```python
import os as _os
_os.environ.setdefault("JAX_PLATFORMS", "cpu")
import jax
import jax.numpy as jnp

def _softmax(x, axis=-1):
    return jax.nn.softmax(x, axis=axis)
def _gelu(x):
    return jax.nn.gelu(x, approximate=True)
def _silu(x):
    return jax.nn.silu(x)
def _sigmoid(x):
    return jax.nn.sigmoid(x)
def _layernorm(x, axis=-1, eps=1e-5):
    m = jnp.mean(x, axis=axis, keepdims=True)
    v = jnp.var(x, axis=axis, keepdims=True)
    return (x - m) / jnp.sqrt(v + eps)
def _scatter_add(tgt, idx, src, axis=0):
    return tgt.at[idx].add(src)
def _segment_sum(src, seg, n):
    return jax.ops.segment_sum(src, seg, n)
class _Rng:
    def __init__(self, key):
        self._k = key
    def _next(self):
        self._k, sub = jax.random.split(self._k)
        return sub
    def normal(self, shape):
        return jax.random.normal(self._next(), shape, dtype=jnp.bfloat16)
    def randint(self, lo, hi, shape):
        return jax.random.randint(self._next(), shape, lo, hi, dtype=jnp.int32)
    def uniform(self, shape, lo=0.0, hi=1.0):
        return jax.random.uniform(self._next(), shape, jnp.bfloat16, lo, hi)
    def permutation(self, n):
        return jax.random.permutation(self._next(), n)


kernel_name = 'standalone__se_block__vision'

def setup_inputs():
    _rng = _Rng(jax.random.key(int.from_bytes(__import__("os").urandom(4), "little")))
    _w = (lambda a: (lambda t: t.astype(jnp.bfloat16) if jnp.issubdtype(t.dtype, jnp.floating) else t)(jnp.asarray(a)))
    H = W = 384
    C = 192; r = max(C // 16, 4)
    return {
        "x": _w((lambda *s: _rng.normal(s) * 0.8)(1, H, W, C)),
        "w_down": _w((lambda *s: _rng.normal(s) * 0.8)(C, r)),
        "w_up": _w((lambda *s: _rng.normal(s) * 0.8)(r, C)),
    }

def reference(x, w_down, w_up):
    s = x.mean(axis=(1, 2))
    s = _sigmoid(_silu(s @ w_down) @ w_up)
    return x * s[:, None, None, :]
```

```python
import jax
import jax.numpy as jnp
from jax import lax
import jax.experimental.pallas as pl
import jax.experimental.pallas.tpu as pltpu

_STREAMS = 6
_PIECE = 48
_LANES = 128
_READS = ((0, 2, 0, 64), (2, 2, 0, 64), (4, 1, 0, 64), (5, 1, 0, 44), (5, 1, 44, 14),
          (5, 1, 58, 4), (5, 1, 62, 1), (5, 1, 63, 1))


def _se_kernel(x_hbm, wd_hbm, wu_hbm, o_hbm, buf, wd_v, wu_v, acc, scale, rsem, wsem,
               osem):
    streams, rows, chans, width = buf.shape
    groups = chans // _PIECE
    tiles = width // _LANES

    def read(i):
        s0, ns, r0, nr = _READS[i]
        idx = (pl.ds(s0, ns), pl.ds(r0, nr))
        return pltpu.make_async_copy(x_hbm.at[idx], buf.at[idx], rsem.at[i])

    for i in range(len(_READS)):
        read(i).start()
    wd_copy = pltpu.make_async_copy(wd_hbm, wd_v, wsem.at[0])
    wu_copy = pltpu.make_async_copy(wu_hbm, wu_v, wsem.at[1])
    wd_copy.start(priority=1)
    wu_copy.start(priority=1)

    acc[...] = jnp.zeros(acc.shape, acc.dtype)

    def accumulate(s0, ns, r0, nr):
        def group(i, _):
            s = s0 + i // groups
            c = pl.ds(pl.multiple_of((i % groups) * _PIECE, _PIECE), _PIECE)

            def row(r, a):
                v = buf[s, r0 + r, c, :].astype(jnp.float32)
                for t in range(tiles):
                    a = a + v[:, t * _LANES:(t + 1) * _LANES]
                return a

            acc[c, :] = lax.fori_loop(0, nr, row, acc[c, :], unroll=min(nr, 2))
            return 0

        lax.fori_loop(0, ns * groups, group, 0)

    for i, chunk in enumerate(_READS):
        read(i).wait()
        if i == 0:
            wd_copy.wait()
            wu_copy.wait()
        accumulate(*chunk)

    total = jnp.sum(acc[...], axis=1, keepdims=True)
    mean = (total * (1.0 / (streams * rows * width))).astype(jnp.bfloat16)
    mean = jnp.broadcast_to(mean, (chans, _LANES))
    hid = jnp.dot(wd_v[...], mean, preferred_element_type=jnp.float32)
    hid = hid.astype(jnp.bfloat16).astype(jnp.float32)
    act = (hid * jax.nn.sigmoid(hid)).astype(jnp.bfloat16)
    gate = lax.dot_general(wu_v[...], act, (((0,), (0,)), ((), ())),
                           preferred_element_type=jnp.float32)
    gate = gate.astype(jnp.bfloat16).astype(jnp.float32)
    scale[...] = jax.nn.sigmoid(gate).astype(jnp.bfloat16).astype(jnp.float32)

    def piece(i, _):
        r = i // groups
        c = pl.ds(pl.multiple_of((i % groups) * _PIECE, _PIECE), _PIECE)
        sc = scale[c, :]
        sc = jnp.concatenate([sc] * tiles, axis=1)
        for s in range(streams):
            buf[s, r, c, :] = (buf[s, r, c, :].astype(jnp.float32) * sc).astype(buf.dtype)
        pltpu.make_async_copy(buf.at[:, r, c, :], o_hbm.at[:, r, c, :], osem).start()
        return 0

    lax.fori_loop(0, rows * groups, piece, 0)
    pltpu.make_async_copy(buf, o_hbm, osem).wait()


@jax.jit
def pallas_standalone__se_block__vision_kernel(
    x: jax.Array,
    w_down: jax.Array,
    w_up: jax.Array,
):
    n, h, w, c = x.shape
    assert n == 1
    view = (_STREAMS, h // _STREAMS, c, w)
    xt = jnp.transpose(x, (0, 1, 3, 2)).reshape(view)
    wdt = w_down.T
    hbm = pl.BlockSpec(memory_space=pltpu.HBM)
    out = pl.pallas_call(
        _se_kernel,
        out_shape=jax.ShapeDtypeStruct(view, x.dtype),
        in_specs=[hbm, hbm, hbm],
        out_specs=hbm,
        scratch_shapes=[
            pltpu.VMEM(view, x.dtype),
            pltpu.VMEM(wdt.shape, wdt.dtype),
            pltpu.VMEM(w_up.shape, w_up.dtype),
            pltpu.VMEM((c, _LANES), jnp.float32),
            pltpu.VMEM((c, _LANES), jnp.float32),
            pltpu.SemaphoreType.DMA((len(_READS),)),
            pltpu.SemaphoreType.DMA((2,)),
            pltpu.SemaphoreType.DMA(()),
        ],
        compiler_params=pltpu.CompilerParams(vmem_limit_bytes=80 * 2**20),
        name="se_block",
    )(xt, wdt, w_up)
    return jnp.transpose(out.reshape(n, h, c, w), (0, 1, 3, 2))
```

```python
import jax
import jax.numpy as jnp
from jax import lax
import jax.experimental.pallas as pl
import jax.experimental.pallas.tpu as pltpu

_LANES = 128
_F32 = jnp.float32
_BF16 = jnp.bfloat16

_LATE = 16
_FULL_READS = ((0, 320),)
_EARLY_READS = ((320, 368), (368, 384))
_LATE_READS = ((320, 372), (372, 384))
_SUM_CHANNELS = 48
_SUM_UNROLL = 8

_STREAM_ROWS = 2048
_PIECE = 8
_GROUPS = ((5, 6), (6, 1))


def _round(v):
    return v.astype(_BF16).astype(_F32)


def _tree_sum(xs):
    while len(xs) > 1:
        xs = [sum(xs[i + 1:i + 2], xs[i]) for i in range(0, len(xs), 2)]
    return xs[0]


def _gcd(a, b):
    while b:
        a, b = b, a % b
    return a


def _reads(chans):
    return ([(a, b, 0, chans) for a, b in _FULL_READS]
            + [(a, b, _LATE, chans - _LATE) for a, b in _EARLY_READS]
            + [(a, b, 0, _LATE) for a, b in _LATE_READS])


def _se_kernel(x_hbm, wd_hbm, wu_hbm, o_hbm,
               buf, wd_v, wu_v, wd_b, wu_b, scale, acc, sems):
    height, chans, width = buf.shape
    hidden = wd_v.shape[0]
    hidden_pad = wd_b.shape[1]
    tiles = width // _LANES
    reads = _reads(chans)
    n_wide = len(reads) - len(_LATE_READS)
    inv_n = 1.0 / (height * width)

    def read(i):
        h0, h1, c0, nc = reads[i]
        idx = (pl.ds(h0, h1 - h0), pl.ds(c0, nc))
        return pltpu.make_async_copy(x_hbm.at[idx], buf.at[idx], sems.at[i])

    wd_copy = pltpu.make_async_copy(wd_hbm, wd_v, sems.at[len(reads)])
    wu_copy = pltpu.make_async_copy(wu_hbm, wu_v, sems.at[len(reads)])
    wd_copy.start()
    wu_copy.start()
    for i in range(len(reads)):
        read(i).start()
    wd_copy.wait()
    wu_copy.wait()

    pad_rows = jnp.zeros((hidden_pad - hidden, _LANES), _F32)
    chan_ids = lax.broadcasted_iota(jnp.int32, (chans, _LANES), 0)
    hidden_ids = lax.broadcasted_iota(jnp.int32, (hidden, _LANES), 0)

    def spread_down(c, _):
        col = jnp.dot(wd_v[...], (chan_ids == c).astype(_BF16),
                      preferred_element_type=_F32)
        wd_b[c] = jnp.concatenate([col, pad_rows], axis=0)
        return 0

    def spread_up(j, _):
        wu_b[j] = lax.dot_general(wu_v[...], (hidden_ids == j).astype(_BF16),
                                  (((0,), (0,)), ((), ())),
                                  preferred_element_type=_F32)
        return 0

    lax.fori_loop(0, _LATE, spread_down, 0)
    lax.fori_loop(0, hidden, spread_up, 0)

    def add_rows(i, c, a):
        h0, h1, _, _ = reads[i]
        unroll = _SUM_UNROLL * _SUM_CHANNELS // a.shape[0]

        def row(r, a):
            v = buf[h0 + r, c, :].astype(_F32)
            return a + _tree_sum(
                [v[:, t * _LANES:(t + 1) * _LANES] for t in range(tiles)])

        return lax.fori_loop(0, h1 - h0, row, a,
                             unroll=True if h1 - h0 <= unroll else unroll)

    def add_chunk(i):
        _, _, c0, nc = reads[i]
        g = _SUM_CHANNELS if nc % _SUM_CHANNELS == 0 else _LATE

        def group(k, _):
            c = pl.ds(pl.multiple_of(c0 + k * g, 8), g)
            start = jnp.zeros((g, _LANES), _F32) if i == 0 else acc[c, :]
            acc[c, :] = add_rows(i, c, start)
            return 0

        lax.fori_loop(0, nc // g, group, 0)

    for i in range(n_wide):
        read(i).wait()
        add_chunk(i)

    early = jnp.sum(acc[pl.ds(_LATE, chans - _LATE), :], axis=1, keepdims=True)
    early = jnp.concatenate(
        [jnp.zeros((_LATE, _LANES), _BF16),
         jnp.broadcast_to((early * inv_n).astype(_BF16), (chans - _LATE, _LANES))],
        axis=0)
    hid = jnp.dot(wd_v[...], early, preferred_element_type=_F32)
    hid = jnp.concatenate([hid, pad_rows], axis=0)

    late = acc[pl.ds(0, _LATE), :]
    for i in range(n_wide, len(reads)):
        read(i).wait()
        late = add_rows(i, pl.ds(0, _LATE), late)

    late = _round(jnp.sum(late, axis=1, keepdims=True) * inv_n)
    late = jnp.broadcast_to(late, (_LATE, _LANES))
    hid = _round(hid + _tree_sum(
        [wd_b[c] * jnp.broadcast_to(late[c:c + 1], (hidden_pad, _LANES))
         for c in range(_LATE)]))
    act = _round(hid * jax.nn.sigmoid(hid))
    act_rows = [jnp.broadcast_to(act[j:j + 1], (_PIECE, _LANES))
                for j in range(hidden)]

    def gate(c0):
        logit = _round(_tree_sum(
            [act_rows[j] * wu_b[j, pl.ds(c0, _PIECE), :] for j in range(hidden)]))
        return _round(jax.nn.sigmoid(logit))

    def keep_gate(c0, s):
        for r in range(c0, scale.shape[0], chans):
            scale[pl.ds(r, _PIECE), :] = s

    streams = buf.reshape(o_hbm.shape)
    shift = _STREAM_ROWS % chans
    period = _gcd(shift, chans)
    out_sem = sems.at[0]

    def emit(a0, count, row, gate_of):
        rows = pl.ds(row, _PIECE)
        for a in range(count):
            s = jnp.concatenate([gate_of(a * shift % chans)] * tiles, axis=1)
            streams[a0 + a, rows, :] = (
                streams[a0 + a, rows, :].astype(_F32) * s).astype(_BF16)
        idx = (pl.ds(a0, count), rows)
        pltpu.make_async_copy(streams.at[idx], o_hbm.at[idx], out_sem).start()

    def emit_kept(a0, count, row, c):
        c = pl.multiple_of(c, _PIECE)
        emit(a0, count, row, lambda off: scale[pl.ds(c + off, _PIECE), :])

    runs = []
    a0 = 0
    for count, n_groups in _GROUPS:
        runs.append((a0, count, n_groups))
        a0 += count * n_groups

    first = {c0: gate(c0) for c0 in range(0, chans, period)}
    emit(0, _GROUPS[0][0], 0, lambda off: first[off])
    for c0, s in first.items():
        keep_gate(c0, s)
    for a0, count, n_groups in runs:
        def head(g, _):
            a = a0 + g * count
            emit_kept(a, count, 0, lax.rem(a * shift, chans))
            return 0

        lax.fori_loop(1 if a0 == 0 else 0, n_groups, head, 0)

    for c0 in range(0, chans, _PIECE):
        if c0 not in first:
            keep_gate(c0, gate(c0))

    for a0, count, n_groups in runs:
        def group(g, _):
            a = a0 + g * count

            def piece(j, c):
                emit_kept(a, count, pl.multiple_of(j * _PIECE, _PIECE), c)
                c = c + _PIECE
                return jnp.where(c >= chans, c - chans, c)

            lax.fori_loop(1, _STREAM_ROWS // _PIECE, piece,
                          lax.rem(a * shift + _PIECE, chans))
            return 0

        lax.fori_loop(0, n_groups, group, 0)

    pltpu.make_async_copy(streams, o_hbm, out_sem).wait()


@jax.jit
def pallas_standalone__se_block__vision_kernel(
    x: jax.Array,
    w_down: jax.Array,
    w_up: jax.Array,
):
    n, h, w, c = x.shape
    hidden = w_up.shape[0]
    n_streams = sum(count * n_groups for count, n_groups in _GROUPS)
    assert n == 1 and h == _LATE_READS[-1][1] and h * c == n_streams * _STREAM_ROWS
    scale_rows = 2 * c - _gcd(_STREAM_ROWS % c, c)
    hbm = pl.BlockSpec(memory_space=pltpu.HBM)
    out = pl.pallas_call(
        _se_kernel,
        out_shape=jax.ShapeDtypeStruct((n_streams, _STREAM_ROWS, w), x.dtype),
        in_specs=[hbm, hbm, hbm],
        out_specs=hbm,
        scratch_shapes=[
            pltpu.VMEM((h, c, w), x.dtype),
            pltpu.VMEM((hidden, c), w_down.dtype),
            pltpu.VMEM((hidden, c), w_up.dtype),
            pltpu.VMEM((_LATE, -(-hidden // 8) * 8, _LANES), _F32),
            pltpu.VMEM((hidden, c, _LANES), _F32),
            pltpu.VMEM((scale_rows, _LANES), _F32),
            pltpu.VMEM((c, _LANES), _F32),
            pltpu.SemaphoreType.DMA((len(_reads(c)) + 1,)),
        ],
        compiler_params=pltpu.CompilerParams(vmem_limit_bytes=80 * 2**20),
        name="se_block",
    )(jnp.transpose(x, (0, 1, 3, 2)).reshape(h, c, w), w_down.T, w_up)
    return jnp.transpose(out.reshape(n, h, c, w), (0, 1, 3, 2))
```

```python
import math

import jax
import jax.numpy as jnp
from jax import lax
import jax.experimental.pallas as pl
import jax.experimental.pallas.tpu as pltpu

_LANES = 128
_SUBLANES = 8
_F32 = jnp.float32
_BF16 = jnp.bfloat16

_LATE = 16
_FULL_READS = ((0, 192), (192, 352))
_EARLY_READS = ((352, 378), (378, 384))
_LATE_READS = ((352, 379), (379, 384))
_READS_IN_FLIGHT = 2
_SUM_CHANNELS = 48
_SUM_UNROLL = 8

_STREAM_ROWS = 2048
_PIECE = 8
_GROUPS = ((5, 6), (6, 1))
_SOON = 3


def _round(v):
    return v.astype(_BF16).astype(_F32)


def _tree_sum(xs):
    while len(xs) > 1:
        xs = [xs[i] + xs[i + 1] if i + 1 < len(xs) else xs[i]
              for i in range(0, len(xs), 2)]
    return xs[0]


def _lane_tiles(v):
    return [v[:, i:i + _LANES] for i in range(0, v.shape[1], _LANES)]


def _se_kernel(x_hbm, wd_hbm, wu_hbm, o_hbm,
               buf, wd_v, wu_v, wu_f, wd_b, wu_b, scale, acc, sems):
    height, chans, width = buf.shape
    hidden = wd_v.shape[0]
    hidden_pad = wd_b.shape[1]
    inv_n = 1.0 / (height * width)
    reads = ([(h0, h1, 0, chans) for h0, h1 in _FULL_READS]
             + [(h0, h1, _LATE, chans - _LATE) for h0, h1 in _EARLY_READS]
             + [(h0, h1, 0, _LATE) for h0, h1 in _LATE_READS])
    n_wide = len(reads) - len(_LATE_READS)

    def read(i):
        h0, h1, c0, nc = reads[i]
        idx = (pl.ds(h0, h1 - h0), pl.ds(c0, nc))
        return pltpu.make_async_copy(x_hbm.at[idx], buf.at[idx],
                                     sems.at[i % _READS_IN_FLIGHT])

    def finish_read(i):
        read(i).wait()
        if i + _READS_IN_FLIGHT < len(reads):
            read(i + _READS_IN_FLIGHT).start()

    last = _READS_IN_FLIGHT - 1
    wd_copy = pltpu.make_async_copy(wd_hbm, wd_v, sems.at[last])
    wu_copy = pltpu.make_async_copy(wu_hbm, wu_v, sems.at[last])
    wd_copy.start()
    wu_copy.start()
    for i in range(last):
        read(i).start()
    wd_copy.wait()
    wu_copy.wait()
    read(last).start()

    pad_rows = jnp.zeros((hidden_pad - hidden, _LANES), _F32)
    wd_f = wd_v[...].astype(_F32)
    for c in range(_LATE):
        wd_b[c] = jnp.concatenate(
            [jnp.broadcast_to(wd_f[:, c:c + 1], (hidden, _LANES)), pad_rows], axis=0)
    wu_f[...] = wu_v[...].astype(_F32)

    def spread_up(j, _):
        wu_b[j] = jnp.broadcast_to(wu_f[pl.ds(j, 1), :], (_LANES, chans)).T
        return 0

    lax.fori_loop(0, hidden, spread_up, 0)

    def add_rows(i, c, a):
        h0, h1, _, _ = reads[i]
        unroll = _SUM_UNROLL * _SUM_CHANNELS // a.shape[0]

        def row(r, a):
            return a + _tree_sum(_lane_tiles(buf[h0 + r, c, :].astype(_F32)))

        return lax.fori_loop(0, h1 - h0, row, a,
                             unroll=True if h1 - h0 < 2 * unroll else unroll)

    def add_chunk(i):
        _, _, c0, nc = reads[i]
        g = _SUM_CHANNELS if nc % _SUM_CHANNELS == 0 else _LATE

        def group(k, _):
            c = pl.ds(pl.multiple_of(c0 + k * g, _SUBLANES), g)
            start = jnp.zeros((g, _LANES), _F32) if i == 0 else acc[c, :]
            acc[c, :] = add_rows(i, c, start)
            return 0

        lax.fori_loop(0, nc // g, group, 0)

    for i in range(n_wide):
        finish_read(i)
        add_chunk(i)

    early = jnp.sum(acc[pl.ds(_LATE, chans - _LATE), :], axis=1, keepdims=True)
    early = jnp.concatenate(
        [jnp.zeros((_LATE, _LANES), _BF16),
         jnp.broadcast_to((early * inv_n).astype(_BF16), (chans - _LATE, _LANES))],
        axis=0)
    hid = jnp.dot(wd_v[...], early, preferred_element_type=_F32)
    hid = jnp.concatenate([hid, pad_rows], axis=0)

    late_chans = pl.ds(0, _LATE)
    late = acc[late_chans, :]
    for i in range(n_wide, len(reads) - 1):
        finish_read(i)
        late = add_rows(i, late_chans, late)
    finish_read(len(reads) - 1)
    late = _tree_sum([late] + [
        t for h in range(*_LATE_READS[-1])
        for t in _lane_tiles(buf[h, late_chans, :].astype(_F32))])

    late = _round(jnp.sum(late, axis=1, keepdims=True) * inv_n)
    late = jnp.broadcast_to(late, (_LATE, _LANES))
    hid = _round(hid + _tree_sum(
        [wd_b[c] * jnp.broadcast_to(late[c:c + 1], (hidden_pad, _LANES))
         for c in range(_LATE)]))
    act = _round(hid * jax.nn.sigmoid(hid))
    act_rows = [jnp.broadcast_to(act[j:j + 1], (_PIECE, _LANES))
                for j in range(hidden)]

    def gate(c0):
        logit = _round(_tree_sum(
            [act_rows[j] * wu_b[j, pl.ds(c0, _PIECE), :] for j in range(hidden)]))
        return _round(jax.nn.sigmoid(logit))

    def keep_gate(c0, s):
        for r in range(c0, scale.shape[0], chans):
            scale[pl.ds(r, _PIECE), :] = s

    streams = buf.reshape(o_hbm.shape)
    shift = _STREAM_ROWS % chans
    period = math.gcd(shift, chans)
    out_sem = sems.at[0]

    def emit(a0, count, row, gate_of):
        rows = pl.ds(row, _PIECE)
        for a in range(count):
            s = jnp.concatenate(
                [gate_of(a * shift % chans)] * (width // _LANES), axis=1)
            streams[a0 + a, rows, :] = (
                streams[a0 + a, rows, :].astype(_F32) * s).astype(_BF16)
        idx = (pl.ds(a0, count), rows)
        pltpu.make_async_copy(streams.at[idx], o_hbm.at[idx], out_sem).start()

    def emit_kept(a0, count, row, c):
        c = pl.multiple_of(c, _PIECE)
        emit(a0, count, row, lambda offset: scale[pl.ds(c + offset, _PIECE), :])

    def emit_pieces(a0, count, lo, hi):
        def piece(j, c):
            emit_kept(a0, count, pl.multiple_of(j * _PIECE, _PIECE), c)
            c = c + _PIECE
            return jnp.where(c >= chans, c - chans, c)

        lax.fori_loop(lo, hi, piece, lax.rem(a0 * shift + lo * _PIECE, chans))

    runs = []
    start = 0
    for count, n_groups in _GROUPS:
        runs.append((start, count, n_groups))
        start += count * n_groups

    first = {c0: gate(c0) for c0 in range(0, chans, period)}
    emit(0, _GROUPS[0][0], 0, lambda offset: first[offset])
    for c0, s in first.items():
        keep_gate(c0, s)
    for start, count, n_groups in runs:
        def head(g, _):
            a0 = start + g * count
            emit_kept(a0, count, 0, lax.rem(a0 * shift, chans))
            return 0

        lax.fori_loop(1 if start == 0 else 0, n_groups, head, 0)

    for c0 in range(0, chans, _PIECE):
        if 0 < c0 % period <= _SOON * _PIECE:
            keep_gate(c0, gate(c0))
    emit_pieces(0, _GROUPS[0][0], 1, 1 + _SOON)
    for c0 in range(0, chans, _PIECE):
        if c0 % period > _SOON * _PIECE:
            keep_gate(c0, gate(c0))

    for start, count, n_groups in runs:
        def group(g, _):
            done = jnp.where(g == 0, 1 + _SOON, 1) if start == 0 else 1
            emit_pieces(start + g * count, count, done, _STREAM_ROWS // _PIECE)
            return 0

        lax.fori_loop(0, n_groups, group, 0)

    pltpu.make_async_copy(streams, o_hbm, out_sem).wait()


@jax.jit
def pallas_standalone__se_block__vision_kernel(
    x: jax.Array,
    w_down: jax.Array,
    w_up: jax.Array,
):
    n, h, w, c = x.shape
    hidden = w_up.shape[0]
    n_streams = sum(count * n_groups for count, n_groups in _GROUPS)
    assert x.dtype == _BF16 and n == 1 and h == _LATE_READS[-1][1]
    assert h * c == n_streams * _STREAM_ROWS and c % _LATE == 0 and w % _LANES == 0
    scale_rows = 2 * c - math.gcd(_STREAM_ROWS % c, c)
    hidden_pad = pl.cdiv(hidden, _SUBLANES) * _SUBLANES
    hbm = pl.BlockSpec(memory_space=pltpu.HBM)
    out = pl.pallas_call(
        _se_kernel,
        out_shape=jax.ShapeDtypeStruct((n_streams, _STREAM_ROWS, w), x.dtype),
        in_specs=[hbm, hbm, hbm],
        out_specs=hbm,
        scratch_shapes=[
            pltpu.VMEM((h, c, w), x.dtype),
            pltpu.VMEM((hidden, c), w_down.dtype),
            pltpu.VMEM((hidden, c), w_up.dtype),
            pltpu.VMEM((hidden, c), _F32),
            pltpu.VMEM((_LATE, hidden_pad, _LANES), _F32),
            pltpu.VMEM((hidden, c, _LANES), _F32),
            pltpu.VMEM((scale_rows, _LANES), _F32),
            pltpu.VMEM((c, _LANES), _F32),
            pltpu.SemaphoreType.DMA((_READS_IN_FLIGHT,)),
        ],
        compiler_params=pltpu.CompilerParams(vmem_limit_bytes=80 * 2**20),
        name="se_block",
    )(jnp.transpose(x, (0, 1, 3, 2)).reshape(h, c, w), w_down.T, w_up)
    return jnp.transpose(out.reshape(n, h, c, w), (0, 1, 3, 2))
```
